```python
import jax
import jax.numpy as jnp

def _softmax(x, axis=-1):
    return jax.nn.softmax(x, axis=axis)

def _gelu(x):
    return jax.nn.gelu(x, approximate=True)

def _silu(x):
    return jax.nn.silu(x)

def _sigmoid(x):
    return jax.nn.sigmoid(x)

def _layernorm(x, axis=-1, eps=1e-05):
    m = jnp.mean(x, axis=axis, keepdims=True)
    v = jnp.var(x, axis=axis, keepdims=True)
    return (x - m) / jnp.sqrt(v + eps)

def _scatter_add(tgt, idx, src, axis=0):
    return tgt.at[idx].add(src)

def _segment_sum(src, seg, n):
    return jax.ops.segment_sum(src, seg, n)

class _Rng:

    def __init__(self, key):
        self._k = key

    def _next(self):
        self._k, sub = jax.random.split(self._k)
        return sub

    def normal(self, shape):
        return jax.random.normal(self._next(), shape, dtype=jnp.bfloat16)

    def randint(self, lo, hi, shape):
        return jax.random.randint(self._next(), shape, lo, hi, dtype=jnp.int32)

    def uniform(self, shape, lo=0.0, hi=1.0):
        return jax.random.uniform(self._next(), shape, jnp.bfloat16, lo, hi)

    def permutation(self, n):
        return jax.random.permutation(self._next(), n)
kernel_name = 'adaLN_cond__sliding_block_cached__glu_gated_glu__decode'

def setup_inputs():
    _rng = _Rng(jax.random.key(int.from_bytes(__import__("os").urandom(4), "little")))
    _w = lambda a: (lambda t: t.astype(jnp.bfloat16) if jnp.issubdtype(t.dtype, jnp.floating) else t)(jnp.asarray(a))

    def _A_setup():
        B, Sq, D = (8, 1, 512)
        Hq, Hkv, Sk, Dh = (32, 32, 4096, 128)
        assert Hq % Hkv == 0, (Hq, Hkv)
        return {'x': _w((lambda *s: _rng.normal(s) * 0.05)(B, Sq, D)), 'k_cache': _w((lambda *s: _rng.normal(s) * 0.05)(B, Hkv, Sk, Dh)), 'v_cache': _w((lambda *s: _rng.normal(s) * 0.05)(B, Hkv, Sk, Dh)), 'wq': _w((lambda *s: _rng.normal(s) * 0.05)(D, Hq * Dh) * D ** (-0.5)), 'wo': _w((lambda *s: _rng.normal(s) * 0.05)(Hq * Dh, D) * (Hq * Dh) ** (-0.5))}
    _A_in = _A_setup()

    def _B_setup():
        B, S, D, F = (8, 1, 512, 1376)
        return {'x': _w((lambda *s: _rng.normal(s) * 0.05)(B, S, D)), 'w_gate': _w((lambda *s: _rng.normal(s) * 0.05)(D, F)), 'w_up': _w((lambda *s: _rng.normal(s) * 0.05)(D, F)), 'w_down': _w((lambda *s: _rng.normal(s) * 0.05)(F, D))}
    _B_in = _B_setup()
    return {'A_x': _A_in['x'], 'A_k_cache': _A_in['k_cache'], 'A_v_cache': _A_in['v_cache'], 'A_wq': _A_in['wq'], 'A_wo': _A_in['wo'], 'B_x': _B_in['x'], 'B_w_gate': _B_in['w_gate'], 'B_w_up': _B_in['w_up'], 'B_w_down': _B_in['w_down'], 'c': _w((lambda *s: _rng.normal(s) * 0.05)(8, 512)), 'w_mod': _w((lambda *s: _rng.normal(s) * 0.05)(512, 6 * 512) * 512 ** (-0.5))}

def reference(A_x, A_k_cache, A_v_cache, A_wq, A_wo, B_x, B_w_gate, B_w_up, B_w_down, c, w_mod):

    def _A_ref(x, k_cache, v_cache, wq, wo):
        B, Sq, D = x.shape
        Hq, Dh = (32, 128)
        Hkv, Sk = (k_cache.shape[1], k_cache.shape[2])
        W = min(4096, max(256, Sk // 4))
        rep = Hq // Hkv
        q = (lambda x, *d: x.transpose(*d))((x @ wq).reshape(B, Sq, Hq, Dh), 0, 2, 1, 3)
        k = jnp.repeat(k_cache[:, :, Sk - W:, :], rep, axis=1)
        v = jnp.repeat(v_cache[:, :, Sk - W:, :], rep, axis=1)
        scores = jnp.einsum('bhqd,bhkd->bhqk', q, k) * Dh ** (-0.5)
        p = _softmax(scores, axis=-1)
        o = jnp.einsum('bhqk,bhkd->bhqd', p, v)
        return (lambda x, *d: x.transpose(*d))(o, 0, 2, 1, 3).reshape(B, Sq, Hq * Dh) @ wo

    def _B_ref(x, w_gate, w_up, w_down):
        g = jnp.einsum('bsd,df->bsf', x, w_gate)
        u = jnp.einsum('bsd,df->bsf', x, w_up)
        h = _sigmoid(g) * u
        return jnp.einsum('bsf,fd->bsd', h, w_down)
    x = A_x
    mod = (_silu(c) @ w_mod).reshape(c.shape[0], 6, 1, -1)
    sa, ca, ga, sb, cb, gb = (mod[:, 0].copy(), mod[:, 1].copy(), mod[:, 2].copy(), mod[:, 3].copy(), mod[:, 4].copy(), mod[:, 5].copy())
    h = _layernorm(x, axis=-1) * (1 + ca) + sa
    x = x + ga * _A_ref(h, A_k_cache, A_v_cache, A_wq, A_wo)
    h = _layernorm(x, axis=-1) * (1 + cb) + sb
    x = x + gb * _B_ref(h, B_w_gate, B_w_up, B_w_down)
    return x
```

```python
import jax
import jax.numpy as jnp
import jax.experimental.pallas as pl
import jax.experimental.pallas.tpu as pltpu

_B, _D, _H, _DH, _SK, _F = 8, 512, 32, 128, 4096, 1376
_W = min(4096, max(256, _SK // 4))
_EPS = 1e-5
_NS = 4
_NT = (((1,), (1,)), ((), ()))


def _layernorm(x):
    m = jnp.mean(x, axis=-1, keepdims=True)
    xc = x - m
    v = jnp.mean(xc * xc, axis=-1, keepdims=True)
    return xc * jax.lax.rsqrt(v + _EPS)


def _kernel(x_hbm, k_hbm, v_hbm, wq_hbm, wo_hbm, wg_hbm, wu_hbm, wd_hbm, c_hbm, wm_hbm,
            o_ref,
            xbuf, cbuf, wm, wq, wo, wg, wu, wd, kbuf, vbuf, qs, mods, acc,
            sems, ksem, vsem):
    f32, bf16 = jnp.float32, jnp.bfloat16

    def kcopy(h, slot):
        return pltpu.make_async_copy(
            k_hbm.at[:, h, pl.ds(_SK - _W, _W), :], kbuf.at[slot], ksem.at[slot])

    def vcopy(h, slot):
        return pltpu.make_async_copy(
            v_hbm.at[:, h, pl.ds(_SK - _W, _W), :], vbuf.at[slot], vsem.at[slot])

    cp_c = pltpu.make_async_copy(c_hbm, cbuf, sems.at[0])
    cp_x = pltpu.make_async_copy(x_hbm, xbuf, sems.at[1])
    cp_wm = pltpu.make_async_copy(wm_hbm, wm, sems.at[2])
    cp_wq = pltpu.make_async_copy(wq_hbm, wq, sems.at[3])
    cp_wo = pltpu.make_async_copy(wo_hbm, wo, sems.at[4])
    cp_wg = pltpu.make_async_copy(wg_hbm, wg, sems.at[5])
    cp_wu = pltpu.make_async_copy(wu_hbm, wu, sems.at[6])
    cp_wd = pltpu.make_async_copy(wd_hbm, wd, sems.at[7])

    cp_wm.start(priority=1)
    cp_c.start()
    cp_x.start()
    cp_wq.start(priority=1)
    kcopy(0, 0).start(priority=0)
    vcopy(0, 0).start(priority=1)
    cp_wo.start(priority=1)
    for i in range(1, _NS):
        kcopy(i, i).start(priority=0)
        vcopy(i, i).start(priority=1)

    cp_c.wait()
    cp_x.wait()
    c = cbuf[...].astype(f32)
    sc = (c * jax.nn.sigmoid(c)).astype(bf16)
    x = xbuf[...].astype(f32)
    cp_wm.wait()
    mod = jnp.dot(sc, wm[...], preferred_element_type=f32)
    mods[...] = mod
    sa, ca = mod[:, 0:_D], mod[:, _D:2 * _D]
    h = (_layernorm(x) * (1.0 + ca) + sa).astype(bf16)
    cp_wq.wait()
    q = jnp.dot(h, wq[...], preferred_element_type=f32)
    for hh in range(_H):
        qs[hh] = q[:, hh * _DH:(hh + 1) * _DH].astype(bf16)
    acc[...] = jnp.zeros((_B, _D), f32)
    cp_wo.wait()

    row_s = jax.lax.broadcasted_iota(jnp.int32, (_B, _W), 0)
    row_o = jax.lax.broadcasted_iota(jnp.int32, (_B, _DH), 0)
    scale = _DH ** -0.5

    def body(hd, carry):
        slot = hd % _NS
        qh = qs[hd]
        kcopy(hd, slot).wait()
        s = None
        for b in range(_B):
            sb = jax.lax.dot_general(qh, kbuf[slot, b], _NT, preferred_element_type=f32)
            s = sb if s is None else jnp.where(row_s == b, sb, s)

        @pl.when(hd + _NS < _H)
        def _():
            kcopy(hd + _NS, slot).start(priority=0)

        s = s * scale
        m = jnp.max(s, axis=-1, keepdims=True)
        p = jnp.exp(s - m)
        l = jnp.sum(p, axis=-1, keepdims=True)
        pb = p.astype(bf16)
        vcopy(hd, slot).wait()
        o = None
        for b in range(_B):
            ob = jnp.dot(pb, vbuf[slot, b], preferred_element_type=f32)
            o = ob if o is None else jnp.where(row_o == b, ob, o)

        @pl.when(hd + _NS < _H)
        def _():
            vcopy(hd + _NS, slot).start(priority=1)

        @pl.when(hd + _NS == _H)
        def _():
            cp_wg.start(priority=1)
            cp_wu.start(priority=1)
            cp_wd.start(priority=1)

        o = (o / l).astype(bf16)
        acc[...] += jnp.dot(o, wo[pl.ds(pl.multiple_of(hd * _DH, _DH), _DH), :],
                            preferred_element_type=f32)
        return carry

    jax.lax.fori_loop(0, _H, body, 0)

    mod = mods[...]
    ga, sb_, cb, gb = (mod[:, 2 * _D:3 * _D], mod[:, 3 * _D:4 * _D],
                       mod[:, 4 * _D:5 * _D], mod[:, 5 * _D:6 * _D])
    x2 = x + ga * acc[...]
    h2 = (_layernorm(x2) * (1.0 + cb) + sb_).astype(bf16)
    cp_wg.wait()
    cp_wu.wait()
    g = jax.lax.dot_general(h2, wg[...], _NT, preferred_element_type=f32)
    u = jax.lax.dot_general(h2, wu[...], _NT, preferred_element_type=f32)
    hm = (jax.nn.sigmoid(g) * u).astype(bf16)
    cp_wd.wait()
    y = jnp.dot(hm, wd[...], preferred_element_type=f32)
    o_ref[...] = (x2 + gb * y).astype(bf16)


@jax.jit
def pallas_adaLN_cond__sliding_block_cached__glu_gated_glu__decode_kernel(
    A_x: jax.Array,
    A_k_cache: jax.Array,
    A_v_cache: jax.Array,
    A_wq: jax.Array,
    A_wo: jax.Array,
    B_x: jax.Array,
    B_w_gate: jax.Array,
    B_w_up: jax.Array,
    B_w_down: jax.Array,
    c: jax.Array,
    w_mod: jax.Array,
):
    del B_x
    bf16 = jnp.bfloat16
    out = pl.pallas_call(
        _kernel,
        in_specs=[pl.BlockSpec(memory_space=pltpu.HBM)] * 10,
        out_specs=pl.BlockSpec(memory_space=pltpu.VMEM),
        out_shape=jax.ShapeDtypeStruct((_B, _D), bf16),
        scratch_shapes=[
            pltpu.VMEM((_B, _D), bf16),
            pltpu.VMEM((_B, _D), bf16),
            pltpu.VMEM((_D, 6 * _D), bf16),
            pltpu.VMEM((_D, _H * _DH), bf16),
            pltpu.VMEM((_H * _DH, _D), bf16),
            pltpu.VMEM((_F, _D), bf16),
            pltpu.VMEM((_F, _D), bf16),
            pltpu.VMEM((_F, _D), bf16),
            pltpu.VMEM((_NS, _B, _W, _DH), bf16),
            pltpu.VMEM((_NS, _B, _W, _DH), bf16),
            pltpu.VMEM((_H, _B, _DH), bf16),
            pltpu.VMEM((_B, 6 * _D), jnp.float32),
            pltpu.VMEM((_B, _D), jnp.float32),
            pltpu.SemaphoreType.DMA((8,)),
            pltpu.SemaphoreType.DMA((_NS,)),
            pltpu.SemaphoreType.DMA((_NS,)),
        ],
        compiler_params=pltpu.CompilerParams(vmem_limit_bytes=100 * 1024 * 1024),
    )(A_x.reshape(_B, _D), A_k_cache, A_v_cache, A_wq, A_wo,
      B_w_gate.T, B_w_up.T, B_w_down, c, w_mod)
    return out.reshape(_B, 1, _D)
```

```python
import jax
import jax.numpy as jnp
import jax.experimental.pallas as pl
import jax.experimental.pallas.tpu as pltpu

_B, _D, _H, _DH, _SK, _F = 8, 512, 32, 128, 4096, 1376
_W = min(4096, max(256, _SK // 4))
_EPS = 1e-5
_T = 128
_NR = _W // _T
_G = 8
_RS = 8
_NS = 4
_PRIO = (1, 1, 1, 0, 1, 1, 1, 0)
_NT = (((1,), (1,)), ((), ()))
_F32, _BF16 = jnp.float32, jnp.bfloat16


def _layernorm(x):
    m = jnp.mean(x, axis=-1, keepdims=True)
    xc = x - m
    v = jnp.mean(xc * xc, axis=-1, keepdims=True)
    return xc * jax.lax.rsqrt(v + _EPS)


def _al(v, m):
    return v if isinstance(v, int) else pl.multiple_of(v, m)


def _ds(i, n):
    return pl.ds(_al(i * n, n), n)


def _kernel(x_hbm, k_hbm, v_hbm, wq_hbm, wo_hbm, wg_hbm, wu_hbm, wd_hbm, c_hbm, wm_hbm,
            o_ref,
            xbuf, cbuf, wm, wq, wo, wg, wu, wd, kbuf, vbuf, qs, os_, sbuf, pbuf, mods,
            ssem, sems):
    B, D, H, DH, T = _B, _D, _H, _DH, _T
    cp_c = pltpu.make_async_copy(c_hbm, cbuf, ssem.at[0])
    cp_x = pltpu.make_async_copy(x_hbm, xbuf, ssem.at[1])

    def same(src, dst, idx):
        return (src.at[idx], dst.at[idx])

    def s_wm(j):
        return [same(wm_hbm, wm, (_ds(u * 4 + j % 4, 16), _ds(j // 4, 1024))) for u in range(_G)]

    def s_wq(j):
        return [same(wq_hbm, wq, (_ds(u * 4 + j % 4, 16), _ds(j // 4, 1024))) for u in range(_G)]

    def s_wo(j):
        return [same(wo_hbm, wo, (_ds(u * 16 + j, 32), slice(None))) for u in range(_G)]

    def rows32(src, dst, c):
        return same(src, dst, (_ds(c, 32), slice(None)))

    def s_gu(j):
        mats = ((wg_hbm, wg), (wu_hbm, wu))
        return [rows32(*mats[(u // 2) % 2], (u // 4) * 20 + (u % 2) * 10 + j) for u in range(_G)]

    def s_kv(a, h, r):
        src, dst = ((k_hbm, kbuf), (v_hbm, vbuf))[a]
        return [(src.at[b, h, pl.ds(_al(_SK - _W + r * T, T), T), :],
                 dst.at[h % _NS, b, _ds(r, T), :]) for b in range(_B)]

    def issue(seg, sem):
        for u, (s, d) in enumerate(seg):
            pltpu.make_async_copy(s, d, sem).start(priority=_PRIO[u])

    def wait(sem, n=_G):
        d = wo.at[pl.ds(0, 32 * n), :]
        pltpu.make_async_copy(d, d, sem).wait()

    def half(j0, seg_fn, do_wait=True):
        def it(j, carry):
            if do_wait:
                wait(sems.at[j0 + j])
            issue(seg_fn(j), sems.at[j0 + j])
            return carry
        jax.lax.fori_loop(0, 4, it, 0)

    def paced(seg_fn, body=None, carry=0):
        def it(j, carry):
            sem = sems.at[(j + 4) % _RS]
            wait(sem)
            issue(seg_fn(j), sem)
            return carry if body is None else body(j, carry)
        return jax.lax.fori_loop(0, 8, it, carry)

    half(0, s_wm, do_wait=False)
    cp_c.start(priority=1)
    cp_x.start(priority=1)
    half(4, s_wq, do_wait=False)
    half(0, lambda j: s_wq(4 + j))
    cp_c.wait()
    cp_x.wait()
    c = cbuf[...].astype(_F32)
    sc = (c * jax.nn.sigmoid(c)).astype(_BF16)
    x = xbuf[...].astype(_F32)
    mod0 = jnp.dot(sc, wm[:, 0:2 * D], preferred_element_type=_F32)
    h1 = (_layernorm(x) * (1.0 + mod0[:, D:2 * D]) + mod0[:, 0:D]).astype(_BF16)
    half(4, lambda j: s_wq(8 + j))
    half(0, lambda j: s_wq(12 + j))
    half(4, lambda j: s_kv(0, 0, j))
    half(0, lambda j: s_kv(0, 0, 4 + j))

    def qproj(first):
        def body(j, carry):
            jj = first + j
            q = jnp.dot(h1, wq[:, _ds(jj, 2 * DH)], preferred_element_type=_F32).astype(_BF16)
            qs[2 * jj] = q[:, :DH]
            qs[2 * jj + 1] = q[:, DH:]
            return carry
        return body

    paced(lambda j: s_kv(1, 0, j), qproj(0))
    paced(lambda j: s_kv(0, 1, j), qproj(8))

    row = jax.lax.broadcasted_iota(jnp.int32, (B, T), 0)
    scale = DH ** -0.5

    def head(h, seg_a, seg_b):
        slot = h % _NS
        q = qs[h]

        def qk(j, m):
            acc = None
            for b in range(B):
                s = jax.lax.dot_general(q, kbuf[slot, b, _ds(j, T), :], _NT,
                                        preferred_element_type=_F32)
                acc = s if acc is None else jnp.where(row == b, s, acc)
            acc = acc * scale
            sbuf[j] = acc
            return jnp.maximum(m, acc)

        m = paced(seg_a, qk, jnp.full((B, T), -jnp.inf, _F32))
        m = jnp.max(m, axis=-1, keepdims=True)
        l = jnp.zeros((B, T), _F32)
        for j in range(_NR):
            p = jnp.exp(sbuf[j] - m)
            l = l + p
            pbuf[j] = p.astype(_BF16)
        l = jnp.sum(l, axis=-1, keepdims=True)

        def pv(j, o):
            p = pbuf[j]
            acc = None
            for b in range(B):
                ob = jnp.dot(p, vbuf[slot, b, _ds(j, T), :], preferred_element_type=_F32)
                acc = ob if acc is None else jnp.where(row == b, ob, acc)
            return o + acc

        o = paced(seg_b, pv, jnp.zeros((B, T), _F32))
        os_[h] = (o / l).astype(_BF16)

    def head_body(h, carry):
        head(h, lambda j: s_kv(1, h + 1, j), lambda j: s_kv(0, h + 2, j))
        return carry

    jax.lax.fori_loop(0, H - 2, head_body, 0)
    head(H - 2, lambda j: s_kv(1, H - 1, j), lambda j: s_wm(4 + j))
    head(H - 1, s_wo, lambda j: s_wo(8 + j))

    mods[...] = jnp.dot(sc, wm[:, 2 * D:6 * D], preferred_element_type=_F32)
    paced(s_gu)
    attn = jnp.zeros((B, D), _F32)
    for hh in range(H):
        attn = attn + jnp.dot(os_[hh], wo[hh * DH:(hh + 1) * DH, :], preferred_element_type=_F32)
    x2 = x + mods[:, 0:D] * attn
    h2 = (_layernorm(x2) * (1.0 + mods[:, 2 * D:3 * D]) + mods[:, D:2 * D]).astype(_BF16)

    rest = s_gu(8) + s_gu(9)
    for cidx in range(40, _F // 32):
        rest += [rows32(wg_hbm, wg, cidx), rows32(wu_hbm, wu, cidx)]
    n_wd = _F // 32
    stride = -(-n_wd // 4)
    wd_order = sorted(range(n_wd), key=lambda t: (t % stride, t))
    wd_desc = [rows32(wd_hbm, wd, t) for t in wd_order]
    todo = [rest[i:i + _G] for i in range(0, len(rest), _G)]
    n_gu_tail = len(todo)
    todo += [wd_desc[i:i + _G] for i in range(0, n_wd, _G)]
    n_wd_seg = len(todo) - n_gu_tail
    pending = [((j + 4) % _RS, _G) for j in range(_RS)]

    def step():
        si, n = pending.pop(0)
        wait(sems.at[si], n)
        if todo:
            seg = todo.pop(0)
            issue(seg, sems.at[si])
            pending.append((si, len(seg)))

    for _ in range(_RS + n_gu_tail):
        step()
    g = jax.lax.dot_general(h2, wg[...], _NT, preferred_element_type=_F32)
    u = jax.lax.dot_general(h2, wu[...], _NT, preferred_element_type=_F32)
    hm = (jax.nn.sigmoid(g) * u).astype(_BF16)
    for _ in range(n_wd_seg):
        step()
    assert not pending and not todo
    y = jnp.dot(hm, wd[...], preferred_element_type=_F32)
    o_ref[...] = (x2 + mods[:, 3 * D:4 * D] * y).astype(_BF16)


@jax.jit
def pallas_adaLN_cond__sliding_block_cached__glu_gated_glu__decode_kernel(
    A_x: jax.Array,
    A_k_cache: jax.Array,
    A_v_cache: jax.Array,
    A_wq: jax.Array,
    A_wo: jax.Array,
    B_x: jax.Array,
    B_w_gate: jax.Array,
    B_w_up: jax.Array,
    B_w_down: jax.Array,
    c: jax.Array,
    w_mod: jax.Array,
):
    del B_x
    B, D, H, DH, F, W, T = _B, _D, _H, _DH, _F, _W, _T
    out = pl.pallas_call(
        _kernel,
        in_specs=[pl.BlockSpec(memory_space=pltpu.HBM)] * 10,
        out_specs=pl.BlockSpec(memory_space=pltpu.VMEM),
        out_shape=jax.ShapeDtypeStruct((B, D), _BF16),
        scratch_shapes=[
            pltpu.VMEM((B, D), _BF16),
            pltpu.VMEM((B, D), _BF16),
            pltpu.VMEM((D, 6 * D), _BF16),
            pltpu.VMEM((D, H * DH), _BF16),
            pltpu.VMEM((H * DH, D), _BF16),
            pltpu.VMEM((F, D), _BF16),
            pltpu.VMEM((F, D), _BF16),
            pltpu.VMEM((F, D), _BF16),
            pltpu.VMEM((_NS, B, W, DH), _BF16),
            pltpu.VMEM((_NS, B, W, DH), _BF16),
            pltpu.VMEM((H, B, DH), _BF16),
            pltpu.VMEM((H, B, DH), _BF16),
            pltpu.VMEM((_NR, B, T), _F32),
            pltpu.VMEM((_NR, B, T), _BF16),
            pltpu.VMEM((B, 4 * D), _F32),
            pltpu.SemaphoreType.DMA((2,)),
            pltpu.SemaphoreType.DMA((_RS,)),
        ],
        compiler_params=pltpu.CompilerParams(
            vmem_limit_bytes=64 * 1024 * 1024, disable_bounds_checks=True),
    )(A_x.reshape(B, D), A_k_cache, A_v_cache, A_wq, A_wo,
      B_w_gate.T, B_w_up.T, B_w_down, c, w_mod)
    return out.reshape(B, 1, D)
```

```python
import jax
import jax.numpy as jnp
import jax.experimental.pallas as pl
import jax.experimental.pallas.tpu as pltpu

_B, _D, _H, _DH, _SK, _F = 8, 512, 32, 128, 4096, 1376
_W = min(4096, max(256, _SK // 4))
_EPS = 1e-5
_T = 128
_NR = _W // _T
_G = 8
_RS = 8
_NS = 4
_PRIO = (1, 0, 1, 1, 0, 1, 1, 0)
_DIAG = 3
_SHIFT = (64, 0)
_NT = (((1,), (1,)), ((), ()))
_F32, _BF16 = jnp.float32, jnp.bfloat16


def _layernorm(x):
    m = jnp.mean(x, axis=-1, keepdims=True)
    xc = x - m
    v = jnp.mean(xc * xc, axis=-1, keepdims=True)
    return xc * jax.lax.rsqrt(v + _EPS)


def _al(v, m):
    return v if isinstance(v, int) else pl.multiple_of(v, m)


def _ds(i, n):
    return pl.ds(_al(i * n, n), n)


def _kernel(x_hbm, k_hbm, v_hbm, wq_hbm, wo_hbm, wg_hbm, wu_hbm, wd_hbm, c_hbm, wm_hbm,
            o_ref,
            xbuf, cbuf, wm, wq, wo, wg, wu, wd, kbuf, vbuf, qs, os_, sbuf, pbuf, mods,
            ssem, sems):
    B, D, H, DH, T = _B, _D, _H, _DH, _T
    cp_c = pltpu.make_async_copy(c_hbm, cbuf, ssem.at[0])
    cp_x = pltpu.make_async_copy(x_hbm, xbuf, ssem.at[1])

    def same(src, dst, idx):
        return (src.at[idx], dst.at[idx])

    def s_wm(j):
        return [same(wm_hbm, wm, (_ds(u * 4 + j % 4, 16), _ds(j // 4, 1024))) for u in range(_G)]

    def s_wq(j):
        return [same(wq_hbm, wq, (_ds(u * 4 + j % 4, 16), _ds(j // 4, 1024))) for u in range(_G)]

    def s_wo(j):
        return [same(wo_hbm, wo, (_ds(u * 16 + j, 32), slice(None))) for u in range(_G)]

    def rows32(src, dst, c):
        return same(src, dst, (_ds(c, 32), slice(None)))

    def s_gu(j):
        mats = ((wg_hbm, wg), (wu_hbm, wu))
        return [rows32(*mats[(u // 2) % 2], (u // 4) * 20 + (u % 2) * 10 + j) for u in range(_G)]

    def s_kv(a, h, j):
        src, dst = ((k_hbm, kbuf), (v_hbm, vbuf))[a]
        slot, sh = h % _NS, _SHIFT[a]

        def piece(b, r0, n):
            return (src.at[b, h, pl.ds(_al(_SK - _W + r0, 16), n), :],
                    dst.at[slot, b, pl.ds(_al(r0, 16), n), :])

        seg = []
        for b in range(_B):
            r = (j + _DIAG * b) & (_NR - 1)
            full = piece(b, sh + r * T, T)
            if sh:
                seg.append((r, full, piece(b, _W - T + sh, T - sh), piece(b, 0, sh)))
            else:
                seg.append(full)
        return seg

    def issue(seg, sem):
        for u, e in enumerate(seg):
            def start(pair, prio):
                pltpu.make_async_copy(pair[0], pair[1], sem).start(priority=prio)
            if len(e) == 2:
                start(e, _PRIO[u])
                continue
            r, full, tail, head_ = e

            @pl.when(r != _NR - 1)
            def _():
                start(full, _PRIO[u])

            @pl.when(r == _NR - 1)
            def _():
                start(tail, _PRIO[u])
                start(head_, 1)

    def wait(sem, n=_G):
        d = wo.at[pl.ds(0, 32 * n), :]
        pltpu.make_async_copy(d, d, sem).wait()

    def half(j0, seg_fn, do_wait=True):
        def it(j, carry):
            if do_wait:
                wait(sems.at[j0 + j])
            issue(seg_fn(j), sems.at[j0 + j])
            return carry
        jax.lax.fori_loop(0, 4, it, 0)

    def paced(seg_fn, body=None, carry=0):
        def it(j, carry):
            sem = sems.at[(j + 4) % _RS]
            wait(sem)
            issue(seg_fn(j), sem)
            return carry if body is None else body(j, carry)
        return jax.lax.fori_loop(0, 8, it, carry)

    half(0, s_wm, do_wait=False)
    cp_c.start(priority=1)
    cp_x.start(priority=1)
    half(4, s_wq, do_wait=False)
    half(0, lambda j: s_wq(4 + j))
    cp_c.wait()
    cp_x.wait()
    c = cbuf[...].astype(_F32)
    sc = (c * jax.nn.sigmoid(c)).astype(_BF16)
    x = xbuf[...].astype(_F32)
    mod0 = jnp.dot(sc, wm[:, 0:2 * D], preferred_element_type=_F32)
    h1 = (_layernorm(x) * (1.0 + mod0[:, D:2 * D]) + mod0[:, 0:D]).astype(_BF16)
    half(4, lambda j: s_wq(8 + j))
    half(0, lambda j: s_wq(12 + j))
    half(4, lambda j: s_kv(0, 0, j))
    half(0, lambda j: s_kv(0, 0, 4 + j))

    def qproj(first):
        def body(j, carry):
            jj = first + j
            q = jnp.dot(h1, wq[:, _ds(jj, 2 * DH)], preferred_element_type=_F32).astype(_BF16)
            qs[2 * jj] = q[:, :DH]
            qs[2 * jj + 1] = q[:, DH:]
            return carry
        return body

    paced(lambda j: s_kv(1, 0, j), qproj(0))
    paced(lambda j: s_kv(0, 1, j), qproj(8))

    row = jax.lax.broadcasted_iota(jnp.int32, (B, T), 0)
    scale = DH ** -0.5

    def head(h, seg_a, seg_b):
        slot = h % _NS
        q = qs[h]

        def qk(j, m):
            acc = None
            for b in range(B):
                s = jax.lax.dot_general(q, kbuf[slot, b, _ds(j, T), :], _NT,
                                        preferred_element_type=_F32)
                acc = s if acc is None else jnp.where(row == b, s, acc)
            acc = acc * scale
            sbuf[j] = acc
            return jnp.maximum(m, acc)

        m = paced(seg_a, qk, jnp.full((B, T), -jnp.inf, _F32))
        m = jnp.max(m, axis=-1, keepdims=True)
        l = jnp.zeros((B, T), _F32)
        for j in range(_NR):
            p = jnp.exp(sbuf[j] - m)
            l = l + p
            pbuf[j] = p.astype(_BF16)
        l = jnp.sum(l, axis=-1, keepdims=True)

        def pv(j, o):
            p = pbuf[j]
            acc = None
            for b in range(B):
                ob = jnp.dot(p, vbuf[slot, b, _ds(j, T), :], preferred_element_type=_F32)
                acc = ob if acc is None else jnp.where(row == b, ob, acc)
            return o + acc

        o = paced(seg_b, pv, jnp.zeros((B, T), _F32))
        os_[h] = (o / l).astype(_BF16)

    def head_body(h, carry):
        head(h, lambda j: s_kv(1, h + 1, j), lambda j: s_kv(0, h + 2, j))
        return carry

    jax.lax.fori_loop(0, H - 2, head_body, 0)
    head(H - 2, lambda j: s_kv(1, H - 1, j), lambda j: s_wm(4 + j))
    head(H - 1, s_wo, lambda j: s_wo(8 + j))

    mods[...] = jnp.dot(sc, wm[:, 2 * D:6 * D], preferred_element_type=_F32)
    paced(s_gu)
    attn = jnp.zeros((B, D), _F32)
    for hh in range(H):
        attn = attn + jnp.dot(os_[hh], wo[hh * DH:(hh + 1) * DH, :], preferred_element_type=_F32)
    x2 = x + mods[:, 0:D] * attn
    h2 = (_layernorm(x2) * (1.0 + mods[:, 2 * D:3 * D]) + mods[:, D:2 * D]).astype(_BF16)

    rest = s_gu(8) + s_gu(9)
    for cidx in range(40, _F // 32):
        rest += [rows32(wg_hbm, wg, cidx), rows32(wu_hbm, wu, cidx)]
    n_wd = _F // 32
    stride = -(-n_wd // 4)
    wd_order = sorted(range(n_wd), key=lambda t: (t % stride, t))
    wd_desc = [rows32(wd_hbm, wd, t) for t in wd_order]
    todo = [rest[i:i + _G] for i in range(0, len(rest), _G)]
    n_gu_tail = len(todo)
    todo += [wd_desc[i:i + _G] for i in range(0, n_wd, _G)]
    n_wd_seg = len(todo) - n_gu_tail
    pending = [((j + 4) % _RS, _G) for j in range(_RS)]

    def step():
        si, n = pending.pop(0)
        wait(sems.at[si], n)
        if todo:
            seg = todo.pop(0)
            issue(seg, sems.at[si])
            pending.append((si, len(seg)))

    for _ in range(_RS + n_gu_tail):
        step()
    g = jax.lax.dot_general(h2, wg[...], _NT, preferred_element_type=_F32)
    u = jax.lax.dot_general(h2, wu[...], _NT, preferred_element_type=_F32)
    hm = (jax.nn.sigmoid(g) * u).astype(_BF16)
    for _ in range(n_wd_seg):
        step()
    assert not pending and not todo
    y = jnp.dot(hm, wd[...], preferred_element_type=_F32)
    o_ref[...] = (x2 + mods[:, 3 * D:4 * D] * y).astype(_BF16)


@jax.jit
def pallas_adaLN_cond__sliding_block_cached__glu_gated_glu__decode_kernel(
    A_x: jax.Array,
    A_k_cache: jax.Array,
    A_v_cache: jax.Array,
    A_wq: jax.Array,
    A_wo: jax.Array,
    B_x: jax.Array,
    B_w_gate: jax.Array,
    B_w_up: jax.Array,
    B_w_down: jax.Array,
    c: jax.Array,
    w_mod: jax.Array,
):
    del B_x
    B, D, H, DH, F, W, T = _B, _D, _H, _DH, _F, _W, _T
    out = pl.pallas_call(
        _kernel,
        in_specs=[pl.BlockSpec(memory_space=pltpu.HBM)] * 10,
        out_specs=pl.BlockSpec(memory_space=pltpu.VMEM),
        out_shape=jax.ShapeDtypeStruct((B, D), _BF16),
        scratch_shapes=[
            pltpu.VMEM((B, D), _BF16),
            pltpu.VMEM((B, D), _BF16),
            pltpu.VMEM((D, 6 * D), _BF16),
            pltpu.VMEM((D, H * DH), _BF16),
            pltpu.VMEM((H * DH, D), _BF16),
            pltpu.VMEM((F, D), _BF16),
            pltpu.VMEM((F, D), _BF16),
            pltpu.VMEM((F, D), _BF16),
            pltpu.VMEM((_NS, B, W, DH), _BF16),
            pltpu.VMEM((_NS, B, W, DH), _BF16),
            pltpu.VMEM((H, B, DH), _BF16),
            pltpu.VMEM((H, B, DH), _BF16),
            pltpu.VMEM((_NR, B, T), _F32),
            pltpu.VMEM((_NR, B, T), _BF16),
            pltpu.VMEM((B, 4 * D), _F32),
            pltpu.SemaphoreType.DMA((2,)),
            pltpu.SemaphoreType.DMA((_RS,)),
        ],
        compiler_params=pltpu.CompilerParams(
            vmem_limit_bytes=64 * 1024 * 1024, disable_bounds_checks=True,
            disable_semaphore_checks=True),
    )(A_x.reshape(B, D), A_k_cache, A_v_cache, A_wq, A_wo,
      B_w_gate.T, B_w_up.T, B_w_down, c, w_mod)
    return out.reshape(B, 1, D)
```

```python
import jax
import jax.numpy as jnp
import jax.experimental.pallas as pl
import jax.experimental.pallas.tpu as pltpu

_B, _D, _H, _DH, _SK, _F = 8, 512, 32, 128, 4096, 1376
_W = min(4096, max(256, _SK // 4))
_EPS = 1e-5

_T = 128
_NR = _W // _T
_G = 8
_PRIO = (1, 0, 1, 1, 0, 1, 1, 0)
_DIAG = 3
_SHIFT = (64, 0)
_GLU_CUTS = (0, 1024, _F)
_NT = (((1,), (1,)), ((), ()))
_F32, _BF16 = jnp.float32, jnp.bfloat16
_WAIT = "wait"


def _layernorm(x):
    m = jnp.mean(x, axis=-1, keepdims=True)
    xc = x - m
    v = jnp.mean(xc * xc, axis=-1, keepdims=True)
    return xc * jax.lax.rsqrt(v + _EPS)


def _al(v, m):
    return v if isinstance(v, int) else pl.multiple_of(v, m)


def _ds(i, n):
    return pl.ds(_al(i * n, n), n)


def _spread(items, ways=4):
    stride = -(-len(items) // ways)
    return [items[t] for t in sorted(range(len(items)), key=lambda t: (t % stride, t))]


def _kernel(x_hbm, k_hbm, v_hbm, wq_hbm, wo_hbm, wg_hbm, wu_hbm, wd_hbm, c_hbm, wm_hbm,
            o_ref,
            xbuf, cbuf, wm, wq, wo, wg, wu, wd, kbuf, vbuf, qs, os_, sbuf, pbuf, mods, hbuf,
            csem, sems):
    B, D, H, DH, T, G = _B, _D, _H, _DH, _T, _G

    def run(src, dst, sem, op):
        cp = pltpu.make_async_copy(src, dst, sem)
        if op == _WAIT:
            cp.wait()
        else:
            cp.start(priority=op)

    def weight(src, dst, idx, sem, op):
        run(src.at[idx], dst.at[idx], sem, op)

    def wm_index(slab, i, u):
        return (_ds(u * 4 + i, 16), _ds(slab, 1024))

    def ph_wm01(j, u, sem, op):
        weight(wm_hbm, wm, wm_index(j // 4, j % 4, u), sem, op)

    def ph_wq(half):
        def phase(j, u, sem, op):
            weight(wq_hbm, wq, (_ds((u // 2) * 8 + j, 16), _ds(half * 2 + u % 2, 1024)), sem, op)
        return phase

    def ph_wo(half):
        def phase(j, u, sem, op):
            weight(wo_hbm, wo, (_ds(half * 8 + u * 16 + j, 32), slice(None)), sem, op)
        return phase

    def ph_kv(a, h):
        src, dst = ((k_hbm, kbuf), (v_hbm, vbuf))[a]
        shift, slot = _SHIFT[a], h % 2

        def phase(j, b, sem, op):
            def rows(r0, n, op):
                run(src.at[b, h, pl.ds(_al(_SK - _W + r0, 16), n), :],
                    dst.at[slot, b, pl.ds(_al(r0, 16), n), :], sem, op)

            r = (j + _DIAG * b) & (_NR - 1)
            if not shift:
                rows(r * T, T, op)
            elif op == _WAIT:
                rows(0, T, op)
            else:
                @pl.when(r != _NR - 1)
                def _():
                    rows(shift + r * T, T, op)

                @pl.when(r == _NR - 1)
                def _():
                    rows(_W - T + shift, T - shift, op)
                    rows(0, shift, 1)
        return phase

    def paced(cur, nxt, body=None, carry=0):
        def step(j, carry):
            for u in range(G):
                cur(j, u, sems.at[j], _WAIT)
            for u in range(G):
                nxt(j, u, sems.at[j], _PRIO[u])
            return carry if body is None else body(j, carry)
        return jax.lax.fori_loop(0, G, step, carry)

    cp_c = pltpu.make_async_copy(c_hbm, cbuf, csem.at[0])
    cp_x = pltpu.make_async_copy(x_hbm, xbuf, csem.at[1])
    cp_c.start(priority=1)
    cp_x.start(priority=1)

    def first(j, carry):
        for u in range(G):
            ph_wm01(j, u, sems.at[j], _PRIO[u])
        return carry

    jax.lax.fori_loop(0, G, first, 0)
    paced(ph_wm01, ph_wq(0))
    cp_c.wait()
    cp_x.wait()
    c = cbuf[...].astype(_F32)
    hbuf[...] = (c * jax.nn.sigmoid(c)).astype(_BF16)

    def mod_slice(j, carry):
        mods[:, _ds(j, 256)] = jnp.dot(hbuf[...], wm[:, _ds(j, 256)],
                                       preferred_element_type=_F32)
        return carry

    paced(ph_wq(0), ph_wq(1), mod_slice)
    x = xbuf[...].astype(_F32)
    hbuf[...] = (_layernorm(x) * (1.0 + mods[:, D:2 * D]) + mods[:, 0:D]).astype(_BF16)
    paced(ph_wq(1), ph_kv(0, 0))

    def q_slice(j, carry):
        for jj in (j, G + j):
            q = jnp.dot(hbuf[...], wq[:, _ds(jj, 2 * DH)],
                        preferred_element_type=_F32).astype(_BF16)
            qs[2 * jj] = q[:, :DH]
            qs[2 * jj + 1] = q[:, DH:]
        return carry

    paced(ph_kv(0, 0), ph_kv(1, 0), q_slice)

    row = jax.lax.broadcasted_iota(jnp.int32, (B, T), 0)
    scale = DH ** -0.5

    def head(h, ph_v, ph_next_k, ph_next_v):
        slot = h % 2
        q = qs[h]

        def qk(j, m):
            acc = None
            for b in range(B):
                s = jax.lax.dot_general(q, kbuf[slot, b, _ds(j, T), :], _NT,
                                        preferred_element_type=_F32)
                acc = s if acc is None else jnp.where(row == b, s, acc)
            acc = acc * scale
            sbuf[j] = acc
            return jnp.maximum(m, acc)

        m = paced(ph_v, ph_next_k, qk, jnp.full((B, T), -jnp.inf, _F32))
        m = jnp.max(m, axis=-1, keepdims=True)
        l = jnp.zeros((B, T), _F32)
        for j in range(_NR):
            p = jnp.exp(sbuf[j] - m)
            l = l + p
            pbuf[j] = p.astype(_BF16)
        l = jnp.sum(l, axis=-1, keepdims=True)

        def pv(j, o):
            p = pbuf[j]
            acc = None
            for b in range(B):
                ob = jnp.dot(p, vbuf[slot, b, _ds(j, T), :], preferred_element_type=_F32)
                acc = ob if acc is None else jnp.where(row == b, ob, acc)
            return o + acc

        o = paced(ph_next_k, ph_next_v, pv, jnp.zeros((B, T), _F32))
        os_[h] = (o / l).astype(_BF16)

    def head_loop(h, carry):
        head(h, ph_kv(1, h), ph_kv(0, h + 1), ph_kv(1, h + 1))
        return carry

    jax.lax.fori_loop(0, H - 1, head_loop, 0)
    head(H - 1, ph_kv(1, H - 1), ph_wo(0), ph_wo(1))

    def chunk(src, dst, t):
        return (src, dst, (pl.ds(t * 32, 32), slice(None)))

    gate_up, gate_up_end = [], []
    down, down_end = [], []
    for lo, hi in zip(_GLU_CUTS, _GLU_CUTS[1:]):
        for t in _spread(list(range(lo // 32, hi // 32))):
            gate_up += [chunk(wg_hbm, wg, t), chunk(wu_hbm, wu, t)]
            down.append(chunk(wd_hbm, wd, t))
        gate_up_end.append(len(gate_up))
        down_end.append(len(down))
    wm2 = [(wm_hbm, wm, wm_index(2, i, u)) for i in range(4) for u in range(G)]
    first_part = wm2 + gate_up
    segs = [None] * G
    segs += [first_part[i:i + G] for i in range(0, len(first_part), G)]
    down_base = len(segs)
    segs += [down[i:i + G] for i in range(0, len(down), G)]
    wo1 = ph_wo(1)
    done = [0]

    def step():
        t = done[0]
        sem = sems.at[t % G]
        if segs[t] is None:
            for u in range(G):
                wo1(t, u, sem, _WAIT)
        else:
            for e in segs[t]:
                weight(*e, sem, _WAIT)
        if t + G < len(segs):
            for u, e in enumerate(segs[t + G]):
                weight(*e, sem, _PRIO[u])
        done[0] += 1

    def land(n):
        while done[0] < n:
            step()

    def out_proj(acc, heads):
        for hh in heads:
            acc = acc + jnp.dot(os_[hh], wo[hh * DH:(hh + 1) * DH, :],
                                preferred_element_type=_F32)
        return acc

    early = [hh for hh in range(H) if hh % 4 < 2]
    late = [hh for hh in range(H) if hh % 4 >= 2]
    attn = jnp.zeros((B, D), _F32)
    for j in range(G):
        land(j + 1)
        attn = out_proj(attn, early[2 * j:2 * j + 2])
    for j in range(2):
        land(G + j + 1)
        attn = out_proj(attn, late[8 * j:8 * j + 8])
    land(G + 5)
    c = cbuf[...].astype(_F32)
    mod2 = jnp.dot((c * jax.nn.sigmoid(c)).astype(_BF16), wm[:, 4 * D:6 * D],
                   preferred_element_type=_F32)
    land(G + 6)
    x2 = xbuf[...].astype(_F32) + mods[:, 2 * D:3 * D] * attn
    h2 = (_layernorm(x2) * (1.0 + mod2[:, 0:D]) + mods[:, 3 * D:4 * D]).astype(_BF16)

    hidden = []
    for lo, hi, end in zip(_GLU_CUTS, _GLU_CUTS[1:], gate_up_end):
        land(G + -(-(len(wm2) + end) // G))
        g = jax.lax.dot_general(h2, wg[lo:hi, :], _NT, preferred_element_type=_F32)
        up = jax.lax.dot_general(h2, wu[lo:hi, :], _NT, preferred_element_type=_F32)
        hidden.append((jax.nn.sigmoid(g) * up).astype(_BF16))
    y = jnp.zeros((B, D), _F32)
    for lo, hi, end, hid in zip(_GLU_CUTS, _GLU_CUTS[1:], down_end, hidden):
        land(down_base + -(-end // G))
        y = y + jnp.dot(hid, wd[lo:hi, :], preferred_element_type=_F32)
    assert done[0] == len(segs)
    o_ref[...] = (x2 + mod2[:, D:2 * D] * y).astype(_BF16)


@jax.jit
def pallas_adaLN_cond__sliding_block_cached__glu_gated_glu__decode_kernel(
    A_x: jax.Array,
    A_k_cache: jax.Array,
    A_v_cache: jax.Array,
    A_wq: jax.Array,
    A_wo: jax.Array,
    B_x: jax.Array,
    B_w_gate: jax.Array,
    B_w_up: jax.Array,
    B_w_down: jax.Array,
    c: jax.Array,
    w_mod: jax.Array,
):
    del B_x
    B, D, H, DH, F, W, T = _B, _D, _H, _DH, _F, _W, _T
    out = pl.pallas_call(
        _kernel,
        in_specs=[pl.BlockSpec(memory_space=pltpu.HBM)] * 10,
        out_specs=pl.BlockSpec(memory_space=pltpu.VMEM),
        out_shape=jax.ShapeDtypeStruct((B, D), _BF16),
        scratch_shapes=[
            pltpu.VMEM((B, D), _BF16),
            pltpu.VMEM((B, D), _BF16),
            pltpu.VMEM((D, 6 * D), _BF16),
            pltpu.VMEM((D, H * DH), _BF16),
            pltpu.VMEM((H * DH, D), _BF16),
            pltpu.VMEM((F, D), _BF16),
            pltpu.VMEM((F, D), _BF16),
            pltpu.VMEM((F, D), _BF16),
            pltpu.VMEM((2, B, W, DH), _BF16),
            pltpu.VMEM((2, B, W, DH), _BF16),
            pltpu.VMEM((H, B, DH), _BF16),
            pltpu.VMEM((H, B, DH), _BF16),
            pltpu.VMEM((_NR, B, T), _F32),
            pltpu.VMEM((_NR, B, T), _BF16),
            pltpu.VMEM((B, 4 * D), _F32),
            pltpu.VMEM((B, D), _BF16),
            pltpu.SemaphoreType.DMA((2,)),
            pltpu.SemaphoreType.DMA((_G,)),
        ],
        compiler_params=pltpu.CompilerParams(
            vmem_limit_bytes=64 * 1024 * 1024,
            disable_bounds_checks=True,
            disable_semaphore_checks=True,
        ),
    )(A_x.reshape(B, D), A_k_cache, A_v_cache, A_wq, A_wo,
      B_w_gate.T, B_w_up.T, B_w_down, c, w_mod)
    return out.reshape(B, 1, D)
```

```python
import jax
import jax.numpy as jnp
import jax.experimental.pallas as pl
import jax.experimental.pallas.tpu as pltpu

_B, _D, _H, _DH, _SK, _F = 8, 512, 32, 128, 4096, 1376
_W = min(4096, max(256, _SK // 4))
_EPS = 1e-5

_T = 128
_NR = _W // _T
_G = 8
_PRIO = (1, 0, 1, 1, 0, 1, 1, 0)
_DIAG = 3
_SHIFT = (64, 0)
_WSHIFT = dict(o=16, g=16, u=16, d=0)
_GLU_CUTS = (0, 896, _F)
_NT = (((1,), (1,)), ((), ()))
_F32, _BF16 = jnp.float32, jnp.bfloat16
_WAIT = "wait"


def _layernorm(x):
    m = jnp.mean(x, axis=-1, keepdims=True)
    xc = x - m
    v = jnp.mean(xc * xc, axis=-1, keepdims=True)
    return xc * jax.lax.rsqrt(v + _EPS)


def _al(v, m):
    return v if isinstance(v, int) else pl.multiple_of(v, m)


def _ds(i, n):
    return pl.ds(_al(i * n, n), n)


def _spread(items, ways=4):
    stride = -(-len(items) // ways)
    return [items[t] for t in sorted(range(len(items)), key=lambda t: (t % stride, t))]


def _kernel(x_hbm, k_hbm, v_hbm, wq_hbm, wo_hbm, wg_hbm, wu_hbm, wd_hbm, c_hbm, wm_hbm,
            o_ref,
            xbuf, cbuf, wm, wq, wo, wg, wu, wd, kbuf, vbuf, qs, os_, sbuf, pbuf, mods, hbuf,
            csem, sems):
    B, D, H, DH, T, G = _B, _D, _H, _DH, _T, _G

    def run(src, dst, sem, op):
        cp = pltpu.make_async_copy(src, dst, sem)
        if op == _WAIT:
            cp.wait()
        else:
            cp.start(priority=op)

    def weight(src, dst, idx, sem, op):
        run(src.at[idx], dst.at[idx], sem, op)

    def wm_index(slab, i, u):
        return (_ds(u * 4 + i, 16), _ds(slab, 1024))

    def ph_wm01(j, u, sem, op):
        weight(wm_hbm, wm, wm_index(j // 4, j % 4, u), sem, op)

    def ph_wq(half):
        def phase(j, u, sem, op):
            weight(wq_hbm, wq, (_ds((u // 2) * 8 + j, 16), _ds(half * 2 + u % 2, 1024)), sem, op)
        return phase

    n_wo = H * DH

    def ph_wo(half):
        shift = _WSHIFT["o"]

        def phase(j, u, sem, op):
            def rows(r0, n, op):
                weight(wo_hbm, wo, (pl.ds(_al(r0, 16), n), slice(None)), sem, op)

            full = (half * 8 + u * 16 + j) * 32 + shift
            if not (shift and half == 1 and u == G - 1):
                rows(full, 32, op)
            elif isinstance(j, int):
                if j < G - 1:
                    rows(full, 32, op)
                else:
                    rows(n_wo - 32 + shift, 32 - shift, op)
                    rows(0, shift, op if op == _WAIT else 1)
            else:
                @pl.when(j < G - 1)
                def _():
                    rows(full, 32, op)

                @pl.when(j == G - 1)
                def _():
                    rows(n_wo - 32 + shift, 32 - shift, op)
                    rows(0, shift, op if op == _WAIT else 1)
        return phase

    def ph_kv(a, h):
        src, dst = ((k_hbm, kbuf), (v_hbm, vbuf))[a]
        shift, slot = _SHIFT[a], h % 2

        def phase(j, b, sem, op):
            def rows(r0, n, op):
                run(src.at[b, h, pl.ds(_al(_SK - _W + r0, 16), n), :],
                    dst.at[slot, b, pl.ds(_al(r0, 16), n), :], sem, op)

            r = (j + _DIAG * b) & (_NR - 1)
            if not shift:
                rows(r * T, T, op)
            elif op == _WAIT:
                rows(0, T, op)
            else:
                @pl.when(r != _NR - 1)
                def _():
                    rows(shift + r * T, T, op)

                @pl.when(r == _NR - 1)
                def _():
                    rows(_W - T + shift, T - shift, op)
                    rows(0, shift, 1)
        return phase

    def paced(cur, nxt, body=None, carry=0):
        def step(j, carry):
            for u in range(G):
                cur(j, u, sems.at[j], _WAIT)
            for u in range(G):
                nxt(j, u, sems.at[j], _PRIO[u])
            return carry if body is None else body(j, carry)
        return jax.lax.fori_loop(0, G, step, carry)

    cp_c = pltpu.make_async_copy(c_hbm, cbuf, csem.at[0])
    cp_x = pltpu.make_async_copy(x_hbm, xbuf, csem.at[1])
    cp_c.start(priority=1)
    cp_x.start(priority=1)

    def first(j, carry):
        for u in range(G):
            ph_wm01(j, u, sems.at[j], _PRIO[u])
        return carry

    jax.lax.fori_loop(0, G, first, 0)
    paced(ph_wm01, ph_wq(0))
    cp_c.wait()
    cp_x.wait()
    c = cbuf[...].astype(_F32)
    hbuf[...] = (c * jax.nn.sigmoid(c)).astype(_BF16)

    def mod_slice(j, carry):
        mods[:, _ds(j, 256)] = jnp.dot(hbuf[...], wm[:, _ds(j, 256)],
                                       preferred_element_type=_F32)
        return carry

    paced(ph_wq(0), ph_wq(1), mod_slice)
    x = xbuf[...].astype(_F32)
    hbuf[...] = (_layernorm(x) * (1.0 + mods[:, D:2 * D]) + mods[:, 0:D]).astype(_BF16)
    paced(ph_wq(1), ph_kv(0, 0))

    def q_slice(j, carry):
        for jj in (j, G + j):
            q = jnp.dot(hbuf[...], wq[:, _ds(jj, 2 * DH)],
                        preferred_element_type=_F32).astype(_BF16)
            qs[2 * jj] = q[:, :DH]
            qs[2 * jj + 1] = q[:, DH:]
        return carry

    paced(ph_kv(0, 0), ph_kv(1, 0), q_slice)

    row = jax.lax.broadcasted_iota(jnp.int32, (B, T), 0)
    scale = DH ** -0.5

    def head(h, ph_v, ph_next_k, ph_next_v):
        slot = h % 2
        q = qs[h]

        def qk(j, m):
            acc = None
            for b in range(B):
                s = jax.lax.dot_general(q, kbuf[slot, b, _ds(j, T), :], _NT,
                                        preferred_element_type=_F32)
                acc = s if acc is None else jnp.where(row == b, s, acc)
            acc = acc * scale
            sbuf[j] = acc
            return jnp.maximum(m, acc)

        m = paced(ph_v, ph_next_k, qk, jnp.full((B, T), -jnp.inf, _F32))
        m = jnp.max(m, axis=-1, keepdims=True)
        l = jnp.zeros((B, T), _F32)
        for j in range(_NR):
            p = jnp.exp(sbuf[j] - m)
            l = l + p
            pbuf[j] = p.astype(_BF16)
        l = jnp.sum(l, axis=-1, keepdims=True)

        def pv(j, o):
            p = pbuf[j]
            acc = None
            for b in range(B):
                ob = jnp.dot(p, vbuf[slot, b, _ds(j, T), :], preferred_element_type=_F32)
                acc = ob if acc is None else jnp.where(row == b, ob, acc)
            return o + acc

        o = paced(ph_next_k, ph_next_v, pv, jnp.zeros((B, T), _F32))
        os_[h] = (o / l).astype(_BF16)

    def head_loop(h, carry):
        head(h, ph_kv(1, h), ph_kv(0, h + 1), ph_kv(1, h + 1))
        return carry

    jax.lax.fori_loop(0, H - 1, head_loop, 0)
    head(H - 1, ph_kv(1, H - 1), ph_wo(0), ph_wo(1))

    def pieces(src, dst, shift):
        buckets = [[] for _ in _GLU_CUTS[1:]]
        for lo in range(shift, _F, 32):
            spans = [(lo, 32)] if lo + 32 <= _F else [(lo, _F - lo), (0, shift)]
            first_row = min(r0 for r0, _ in spans)
            c = min(i for i, end in enumerate(_GLU_CUTS[1:]) if first_row < end)
            buckets[c].append([(src, dst, (pl.ds(r0, n), slice(None))) for r0, n in spans])
        return [_spread(b) for b in buckets]

    gate_up, gate_up_end = [], []
    down, down_end = [], []
    for pg, pu, pd in zip(pieces(wg_hbm, wg, _WSHIFT["g"]), pieces(wu_hbm, wu, _WSHIFT["u"]),
                          pieces(wd_hbm, wd, _WSHIFT["d"])):
        for i in range(max(len(pg), len(pu))):
            gate_up += pg[i:i + 1] + pu[i:i + 1]
        down += pd
        gate_up_end.append(len(gate_up))
        down_end.append(len(down))
    wm2 = [[(wm_hbm, wm, wm_index(2, i, u))] for i in range(4) for u in range(G)]
    first_part = wm2 + gate_up
    segs = [None] * G
    segs += [first_part[i:i + G] for i in range(0, len(first_part), G)]
    down_base = len(segs)
    segs += [down[i:i + G] for i in range(0, len(down), G)]
    wo1 = ph_wo(1)
    done = [0]

    def step():
        t = done[0]
        sem = sems.at[t % G]
        if segs[t] is None:
            for u in range(G):
                wo1(t, u, sem, _WAIT)
        else:
            for unit in segs[t]:
                for e in unit:
                    weight(*e, sem, _WAIT)
        if t + G < len(segs):
            for u, unit in enumerate(segs[t + G]):
                for i, e in enumerate(unit):
                    weight(*e, sem, 1 if i else _PRIO[u])
        done[0] += 1

    def land(n):
        while done[0] < n:
            step()

    def out_proj(acc, heads):
        for hh in heads:
            acc = acc + jnp.dot(os_[hh], wo[hh * DH:(hh + 1) * DH, :],
                                preferred_element_type=_F32)
        return acc

    early = [hh for hh in range(H) if hh % 4 < 2]
    late = [hh for hh in range(H) if hh % 4 >= 2]
    attn = jnp.zeros((B, D), _F32)
    for j in range(G):
        land(j + 1)
        attn = out_proj(attn, early[2 * j:2 * j + 2])
    for j in range(2):
        land(G + j + 1)
        attn = out_proj(attn, late[8 * j:8 * j + 8])
    land(G + 5)
    c = cbuf[...].astype(_F32)
    mod2 = jnp.dot((c * jax.nn.sigmoid(c)).astype(_BF16), wm[:, 4 * D:6 * D],
                   preferred_element_type=_F32)
    land(G + 6)
    x2 = xbuf[...].astype(_F32) + mods[:, 2 * D:3 * D] * attn
    h2 = (_layernorm(x2) * (1.0 + mod2[:, 0:D]) + mods[:, 3 * D:4 * D]).astype(_BF16)

    hidden = []
    for lo, hi, end in zip(_GLU_CUTS, _GLU_CUTS[1:], gate_up_end):
        land(G + -(-(len(wm2) + end) // G))
        g = jax.lax.dot_general(h2, wg[lo:hi, :], _NT, preferred_element_type=_F32)
        up = jax.lax.dot_general(h2, wu[lo:hi, :], _NT, preferred_element_type=_F32)
        hidden.append((jax.nn.sigmoid(g) * up).astype(_BF16))
    for lo, hi, end, hid in zip(_GLU_CUTS, _GLU_CUTS[1:], down_end, hidden):
        land(down_base + -(-end // G))
        x2 = x2 + mod2[:, D:2 * D] * jnp.dot(hid, wd[lo:hi, :], preferred_element_type=_F32)
    assert done[0] == len(segs)
    o_ref[...] = x2.astype(_BF16)


@jax.jit
def pallas_adaLN_cond__sliding_block_cached__glu_gated_glu__decode_kernel(
    A_x: jax.Array,
    A_k_cache: jax.Array,
    A_v_cache: jax.Array,
    A_wq: jax.Array,
    A_wo: jax.Array,
    B_x: jax.Array,
    B_w_gate: jax.Array,
    B_w_up: jax.Array,
    B_w_down: jax.Array,
    c: jax.Array,
    w_mod: jax.Array,
):
    del B_x
    B, D, H, DH, F, W, T = _B, _D, _H, _DH, _F, _W, _T
    out = pl.pallas_call(
        _kernel,
        in_specs=[pl.BlockSpec(memory_space=pltpu.HBM)] * 10,
        out_specs=pl.BlockSpec(memory_space=pltpu.VMEM),
        out_shape=jax.ShapeDtypeStruct((B, D), _BF16),
        scratch_shapes=[
            pltpu.VMEM((B, D), _BF16),
            pltpu.VMEM((B, D), _BF16),
            pltpu.VMEM((D, 6 * D), _BF16),
            pltpu.VMEM((D, H * DH), _BF16),
            pltpu.VMEM((H * DH, D), _BF16),
            pltpu.VMEM((F, D), _BF16),
            pltpu.VMEM((F, D), _BF16),
            pltpu.VMEM((F, D), _BF16),
            pltpu.VMEM((2, B, W, DH), _BF16),
            pltpu.VMEM((2, B, W, DH), _BF16),
            pltpu.VMEM((H, B, DH), _BF16),
            pltpu.VMEM((H, B, DH), _BF16),
            pltpu.VMEM((_NR, B, T), _F32),
            pltpu.VMEM((_NR, B, T), _BF16),
            pltpu.VMEM((B, 4 * D), _F32),
            pltpu.VMEM((B, D), _BF16),
            pltpu.SemaphoreType.DMA((2,)),
            pltpu.SemaphoreType.DMA((_G,)),
        ],
        compiler_params=pltpu.CompilerParams(
            vmem_limit_bytes=64 * 1024 * 1024,
            disable_bounds_checks=True,
            disable_semaphore_checks=True,
        ),
    )(A_x.reshape(B, D), A_k_cache, A_v_cache, A_wq, A_wo,
      B_w_gate.T, B_w_up.T, B_w_down, c, w_mod)
    return out.reshape(B, 1, D)
```

```python
import jax
import jax.numpy as jnp
import jax.experimental.pallas as pl
import jax.experimental.pallas.tpu as pltpu

_B, _D, _H, _DH, _SK, _F = 8, 512, 32, 128, 4096, 1376
_W = min(4096, max(256, _SK // 4))
_EPS = 1e-5

_T = 128
_NR = _W // _T
_G = 8
_PRIO = (1, 0, 1, 1, 0, 1, 1, 0)
_DIAG = 3
_SHIFT = (64, 0)
_WSHIFT = dict(o=16, g=16, u=16, d=0)
_GLU_CUTS = (0, 896, _F)
_NT = (((1,), (1,)), ((), ()))
_F32, _BF16 = jnp.float32, jnp.bfloat16
_WAIT = "wait"


def _layernorm(x):
    m = jnp.mean(x, axis=-1, keepdims=True)
    xc = x - m
    v = jnp.mean(xc * xc, axis=-1, keepdims=True)
    return xc * jax.lax.rsqrt(v + _EPS)


def _al(v, m):
    return v if isinstance(v, int) else pl.multiple_of(v, m)


def _ds(i, n):
    return pl.ds(_al(i * n, n), n)


def _spread(items, ways=4):
    stride = -(-len(items) // ways)
    return [items[t] for t in sorted(range(len(items)), key=lambda t: (t % stride, t))]


def _kernel(x_hbm, k_hbm, v_hbm, wq_hbm, wo_hbm, wg_hbm, wu_hbm, wd_hbm, c_hbm, wm_hbm,
            o_ref,
            xbuf, cbuf, wm, wq, wo, wg, wu, wd, kbuf, vbuf, qs, os_, sbuf, pbuf, mods, hbuf,
            csem, sems):
    B, D, H, DH, T, G = _B, _D, _H, _DH, _T, _G

    def run(src, dst, sem, op):
        cp = pltpu.make_async_copy(src, dst, sem)
        if op == _WAIT:
            cp.wait()
        else:
            cp.start(priority=op)

    def weight(src, dst, idx, sem, op):
        run(src.at[idx], dst.at[idx], sem, op)

    def wm_index(slab, i, u):
        return (_ds(u * 4 + i, 16), _ds(slab, 1024))

    def ph_wm01(j, u, sem, op):
        weight(wm_hbm, wm, wm_index(j // 4, j % 4, u), sem, op)

    def ph_wq(half):
        def phase(j, u, sem, op):
            weight(wq_hbm, wq, (_ds((u // 2) * 8 + j, 16), _ds(half * 2 + u % 2, 1024)), sem, op)
        return phase

    n_wo = H * DH

    def ph_wo(half):
        shift = _WSHIFT["o"]

        def phase(j, u, sem, op):
            def rows(r0, n, op):
                weight(wo_hbm, wo, (pl.ds(_al(r0, 16), n), slice(None)), sem, op)

            full = (half * 8 + u * 16 + j) * 32 + shift
            if not (shift and half == 1 and u == G - 1):
                rows(full, 32, op)
            elif isinstance(j, int):
                if j < G - 1:
                    rows(full, 32, op)
                else:
                    rows(n_wo - 32 + shift, 32 - shift, op)
                    rows(0, shift, op if op == _WAIT else 1)
            else:
                @pl.when(j < G - 1)
                def _():
                    rows(full, 32, op)

                @pl.when(j == G - 1)
                def _():
                    rows(n_wo - 32 + shift, 32 - shift, op)
                    rows(0, shift, op if op == _WAIT else 1)
        return phase

    def ph_kv(a, h):
        src, dst = ((k_hbm, kbuf), (v_hbm, vbuf))[a]
        shift, slot = _SHIFT[a], h % 2

        def phase(j, b, sem, op):
            def rows(r0, n, op):
                run(src.at[b, h, pl.ds(_al(_SK - _W + r0, 16), n), :],
                    dst.at[slot, b, pl.ds(_al(r0, 16), n), :], sem, op)

            r = (j + _DIAG * b) & (_NR - 1)
            if not shift:
                rows(r * T, T, op)
            elif op == _WAIT:
                rows(0, T, op)
            else:
                @pl.when(r != _NR - 1)
                def _():
                    rows(shift + r * T, T, op)

                @pl.when(r == _NR - 1)
                def _():
                    rows(_W - T + shift, T - shift, op)
                    rows(0, shift, 1)
        return phase

    def paced(cur, nxt, body=None, carry=0):
        def step(j, carry):
            for u in range(G):
                cur(j, u, sems.at[j], _WAIT)
            for u in range(G):
                nxt(j, u, sems.at[j], _PRIO[u])
            return carry if body is None else body(j, carry)
        return jax.lax.fori_loop(0, G, step, carry)

    cp_c = pltpu.make_async_copy(c_hbm, cbuf, csem.at[0])
    cp_x = pltpu.make_async_copy(x_hbm, xbuf, csem.at[1])
    cp_c.start(priority=1)
    cp_x.start(priority=1)

    def first(j, carry):
        for u in range(G):
            ph_wm01(j, u, sems.at[j], _PRIO[u])
        return carry

    jax.lax.fori_loop(0, G, first, 0)
    paced(ph_wm01, ph_wq(0))
    cp_c.wait()
    cp_x.wait()
    c = cbuf[...].astype(_F32)
    hbuf[...] = (c * jax.nn.sigmoid(c)).astype(_BF16)

    def mod_slice(j, carry):
        mods[:, _ds(j, 256)] = jnp.dot(hbuf[...], wm[:, _ds(j, 256)],
                                       preferred_element_type=_F32)
        return carry

    paced(ph_wq(0), ph_wq(1), mod_slice)
    x = xbuf[...].astype(_F32)
    hbuf[...] = (_layernorm(x) * (1.0 + mods[:, D:2 * D]) + mods[:, 0:D]).astype(_BF16)
    paced(ph_wq(1), ph_kv(0, 0))

    def q_slice(j, carry):
        for jj in (j, G + j):
            q = jnp.dot(hbuf[...], wq[:, _ds(jj, 2 * DH)],
                        preferred_element_type=_F32).astype(_BF16)
            qs[2 * jj] = q[:, :DH]
            qs[2 * jj + 1] = q[:, DH:]
        return carry

    paced(ph_kv(0, 0), ph_kv(1, 0), q_slice)

    row = jax.lax.broadcasted_iota(jnp.int32, (B, T), 0)
    scale = DH ** -0.5

    def head(h, ph_v, ph_next_k, ph_next_v):
        slot = h % 2
        q = qs[h]

        def qk(j, m):
            acc = None
            for b in range(B):
                s = jax.lax.dot_general(q, kbuf[slot, b, _ds(j, T), :], _NT,
                                        preferred_element_type=_F32)
                acc = s if acc is None else jnp.where(row == b, s, acc)
            acc = acc * scale
            sbuf[j] = acc
            return jnp.maximum(m, acc)

        m = paced(ph_v, ph_next_k, qk, jnp.full((B, T), -jnp.inf, _F32))
        m = jnp.max(m, axis=-1, keepdims=True)
        l = jnp.zeros((B, T), _F32)
        for j in range(_NR):
            p = jnp.exp(sbuf[j] - m)
            l = l + p
            pbuf[j] = p.astype(_BF16)
        l = jnp.sum(l, axis=-1, keepdims=True)

        def pv(j, o):
            p = pbuf[j]
            acc = None
            for b in range(B):
                ob = jnp.dot(p, vbuf[slot, b, _ds(j, T), :], preferred_element_type=_F32)
                acc = ob if acc is None else jnp.where(row == b, ob, acc)
            return o + acc

        o = paced(ph_next_k, ph_next_v, pv, jnp.zeros((B, T), _F32))
        os_[h] = (o / l).astype(_BF16)

    def head_loop(h, carry):
        head(h, ph_kv(1, h), ph_kv(0, h + 1), ph_kv(1, h + 1))
        return carry

    jax.lax.fori_loop(0, H - 1, head_loop, 0)
    head(H - 1, ph_kv(1, H - 1), ph_wo(0), ph_wo(1))

    def pieces(src, dst, shift):
        buckets = [[] for _ in _GLU_CUTS[1:]]
        for lo in range(shift, _F, 32):
            spans = [(lo, 32)] if lo + 32 <= _F else [(lo, _F - lo), (0, shift)]
            first_row = min(r0 for r0, _ in spans)
            c = min(i for i, end in enumerate(_GLU_CUTS[1:]) if first_row < end)
            buckets[c].append([(src, dst, (pl.ds(r0, n), slice(None))) for r0, n in spans])
        return [_spread(b) for b in buckets]

    gate_up, gate_up_end = [], []
    down, down_end = [], []
    for pg, pu, pd in zip(pieces(wg_hbm, wg, _WSHIFT["g"]), pieces(wu_hbm, wu, _WSHIFT["u"]),
                          pieces(wd_hbm, wd, _WSHIFT["d"])):
        for i in range(max(len(pg), len(pu))):
            gate_up += pg[i:i + 1] + pu[i:i + 1]
        down += pd
        gate_up_end.append(len(gate_up))
        down_end.append(len(down))
    wm2 = [[(wm_hbm, wm, wm_index(2, i, u))] for i in range(4) for u in range(G)]
    first_part = wm2 + gate_up
    segs = [None] * G
    segs += [first_part[i:i + G] for i in range(0, len(first_part), G)]
    down_base = len(segs)
    segs += [down[i:i + G] for i in range(0, len(down), G)]
    wo1 = ph_wo(1)
    done = [0]

    def step():
        t = done[0]
        sem = sems.at[t % G]
        if segs[t] is None:
            for u in range(G):
                wo1(t, u, sem, _WAIT)
        else:
            for unit in segs[t]:
                for e in unit:
                    weight(*e, sem, _WAIT)
        if t + G < len(segs):
            for u, unit in enumerate(segs[t + G]):
                for i, e in enumerate(unit):
                    weight(*e, sem, 1 if i else _PRIO[u])
        done[0] += 1

    def land(n):
        while done[0] < n:
            step()

    def out_proj(acc, heads):
        for hh in heads:
            acc = acc + jnp.dot(os_[hh], wo[hh * DH:(hh + 1) * DH, :],
                                preferred_element_type=_F32)
        return acc

    def in_first_half(hh):
        shift = _WSHIFT["o"]
        return all(((r - shift) % n_wo // 32) % 16 < 8 for r in range(hh * DH, (hh + 1) * DH))

    early = [hh for hh in range(H) if in_first_half(hh)]
    late = [hh for hh in range(H) if not in_first_half(hh)]
    attn = jnp.zeros((B, D), _F32)
    for j in range(G):
        land(j + 1)
        attn = out_proj(attn, early[j::G])
    for j in range(3):
        land(G + j + 1)
        attn = out_proj(attn, late[j::3])
    land(G + 5)
    c = cbuf[...].astype(_F32)
    mod2 = jnp.dot((c * jax.nn.sigmoid(c)).astype(_BF16), wm[:, 4 * D:6 * D],
                   preferred_element_type=_F32)
    land(G + 6)
    x2 = xbuf[...].astype(_F32) + mods[:, 2 * D:3 * D] * attn
    h2 = (_layernorm(x2) * (1.0 + mod2[:, 0:D]) + mods[:, 3 * D:4 * D]).astype(_BF16)

    hidden = []
    for lo, hi, end in zip(_GLU_CUTS, _GLU_CUTS[1:], gate_up_end):
        land(G + -(-(len(wm2) + end) // G))
        g = jax.lax.dot_general(h2, wg[lo:hi, :], _NT, preferred_element_type=_F32)
        up = jax.lax.dot_general(h2, wu[lo:hi, :], _NT, preferred_element_type=_F32)
        hidden.append((jax.nn.sigmoid(g) * up).astype(_BF16))
    for lo, hi, end, hid in zip(_GLU_CUTS, _GLU_CUTS[1:], down_end, hidden):
        land(down_base + -(-end // G))
        x2 = x2 + mod2[:, D:2 * D] * jnp.dot(hid, wd[lo:hi, :], preferred_element_type=_F32)
    assert done[0] == len(segs)
    o_ref[...] = x2.astype(_BF16)


@jax.jit
def pallas_adaLN_cond__sliding_block_cached__glu_gated_glu__decode_kernel(
    A_x: jax.Array,
    A_k_cache: jax.Array,
    A_v_cache: jax.Array,
    A_wq: jax.Array,
    A_wo: jax.Array,
    B_x: jax.Array,
    B_w_gate: jax.Array,
    B_w_up: jax.Array,
    B_w_down: jax.Array,
    c: jax.Array,
    w_mod: jax.Array,
):
    del B_x
    B, D, H, DH, F, W, T = _B, _D, _H, _DH, _F, _W, _T
    out = pl.pallas_call(
        _kernel,
        in_specs=[pl.BlockSpec(memory_space=pltpu.HBM)] * 10,
        out_specs=pl.BlockSpec(memory_space=pltpu.VMEM),
        out_shape=jax.ShapeDtypeStruct((B, D), _BF16),
        scratch_shapes=[
            pltpu.VMEM((B, D), _BF16),
            pltpu.VMEM((B, D), _BF16),
            pltpu.VMEM((D, 6 * D), _BF16),
            pltpu.VMEM((D, H * DH), _BF16),
            pltpu.VMEM((H * DH, D), _BF16),
            pltpu.VMEM((F, D), _BF16),
            pltpu.VMEM((F, D), _BF16),
            pltpu.VMEM((F, D), _BF16),
            pltpu.VMEM((2, B, W, DH), _BF16),
            pltpu.VMEM((2, B, W, DH), _BF16),
            pltpu.VMEM((H, B, DH), _BF16),
            pltpu.VMEM((H, B, DH), _BF16),
            pltpu.VMEM((_NR, B, T), _F32),
            pltpu.VMEM((_NR, B, T), _BF16),
            pltpu.VMEM((B, 4 * D), _F32),
            pltpu.VMEM((B, D), _BF16),
            pltpu.SemaphoreType.DMA((2,)),
            pltpu.SemaphoreType.DMA((_G,)),
        ],
        compiler_params=pltpu.CompilerParams(
            vmem_limit_bytes=64 * 1024 * 1024,
            disable_bounds_checks=True,
            disable_semaphore_checks=True,
        ),
    )(A_x.reshape(B, D), A_k_cache, A_v_cache, A_wq, A_wo,
      B_w_gate.T, B_w_up.T, B_w_down, c, w_mod)
    return out.reshape(B, 1, D)
```
